```python
import os as _os
_os.environ.setdefault("JAX_PLATFORMS", "cpu")
import jax
import jax.numpy as jnp

def _softmax(x, axis=-1):
    return jax.nn.softmax(x, axis=axis)
def _gelu(x):
    return jax.nn.gelu(x, approximate=True)
def _silu(x):
    return jax.nn.silu(x)
def _sigmoid(x):
    return jax.nn.sigmoid(x)
def _layernorm(x, axis=-1, eps=1e-5):
    m = jnp.mean(x, axis=axis, keepdims=True)
    v = jnp.var(x, axis=axis, keepdims=True)
    return (x - m) / jnp.sqrt(v + eps)
def _scatter_add(tgt, idx, src, axis=0):
    return tgt.at[idx].add(src)
def _segment_sum(src, seg, n):
    return jax.ops.segment_sum(src, seg, n)
class _Rng:
    def __init__(self, key):
        self._k = key
    def _next(self):
        self._k, sub = jax.random.split(self._k)
        return sub
    def normal(self, shape):
        return jax.random.normal(self._next(), shape, dtype=jnp.bfloat16)
    def randint(self, lo, hi, shape):
        return jax.random.randint(self._next(), shape, lo, hi, dtype=jnp.int32)
    def uniform(self, shape, lo=0.0, hi=1.0):
        return jax.random.uniform(self._next(), shape, jnp.bfloat16, lo, hi)
    def permutation(self, n):
        return jax.random.permutation(self._next(), n)


kernel_name = 'concat_heads__softmax_full_mha__softmax_full_mha__prompt'

def setup_inputs():
    _rng = _Rng(jax.random.key(int.from_bytes(__import__("os").urandom(4), "little")))
    _w = (lambda a: (lambda t: t.astype(jnp.bfloat16) if jnp.issubdtype(t.dtype, jnp.floating) else t)(jnp.asarray(a)))
    def _A_setup():
        B, S, D = 1, 2048, 512
        return {
            "x": _w((lambda *s: _rng.normal(s) * 0.2)(B, S, D)),
            "wqkv": _w((lambda *s: _rng.normal(s) * 0.2)(D, 3 * D)),
            "wo": _w((lambda *s: _rng.normal(s) * 0.05)(D, D)),
        }
    _A_in = _A_setup()

    def _B_setup():
        B, S, D = 1, 2048, 512
        return {
            "x": _w((lambda *s: _rng.normal(s) * 0.2)(B, S, D)),
            "wqkv": _w((lambda *s: _rng.normal(s) * 0.2)(D, 3 * D)),
            "wo": _w((lambda *s: _rng.normal(s) * 0.05)(D, D)),
        }
    _B_in = _B_setup()

    return {
        "A_x": _A_in["x"],
        "A_wqkv": _A_in["wqkv"],
        "A_wo": _A_in["wo"],
        "B_x": _B_in["x"],
        "B_wqkv": _B_in["wqkv"],
        "B_wo": _B_in["wo"],
    }

def reference(A_x, A_wqkv, A_wo, B_x, B_wqkv, B_wo):
    def _A_ref(x, wqkv, wo):
        B, S, D = x.shape
        H = 32; Dh = D // H
        qkv = (lambda x, *d: x.transpose(*d))((x @ wqkv).reshape(B, S, 3, H, Dh), 2, 0, 3, 1, 4)
        q, k, v = qkv[0], qkv[1], qkv[2]
        scale = Dh ** -0.5
        scores = jnp.einsum("bhqd,bhkd->bhqk", q, k) * scale
        p = _softmax(scores, axis=-1)
        o = jnp.einsum("bhqk,bhkd->bhqd", p, v)
        return (lambda x, *d: x.transpose(*d))(o, 0, 2, 1, 3).reshape(B, S, D) @ wo

    def _B_ref(x, wqkv, wo):
        B, S, D = x.shape
        H = 32; Dh = D // H
        qkv = (lambda x, *d: x.transpose(*d))((x @ wqkv).reshape(B, S, 3, H, Dh), 2, 0, 3, 1, 4)
        q, k, v = qkv[0], qkv[1], qkv[2]
        scale = Dh ** -0.5
        scores = jnp.einsum("bhqd,bhkd->bhqk", q, k) * scale
        p = _softmax(scores, axis=-1)
        o = jnp.einsum("bhqk,bhkd->bhqd", p, v)
        return (lambda x, *d: x.transpose(*d))(o, 0, 2, 1, 3).reshape(B, S, D) @ wo

    a = _A_ref(A_x, A_wqkv, A_wo)
    b = _B_ref(B_x, B_wqkv, B_wo)
    return jnp.concatenate([a, b], axis=-1)
```

```python
import math

import jax
import jax.numpy as jnp
from jax import lax
import jax.experimental.pallas as pl
import jax.experimental.pallas.tpu as pltpu

S, D, H, DH = 2048, 512, 32, 16
LOG2E = math.log2(math.e)
F32, BF16, U32 = jnp.float32, jnp.bfloat16, jnp.uint32
TQ = 512
NQ = S // TQ
NT = S // 128
NL = TQ // 128
NUN = 2 * NQ
VR = 16
TO = 128
NFLAG = 4
SAFE_LOG2 = 80.0

DLY, LEAD, ROT, HEAD, FIRST, CRAW = 8, 13, 12, 2, 8, 2
KSTART, QSTART, QOFF, KMARGIN = 20, 11, 3, 8


def _schedule():
    stream, pv_at = [], {}
    for i in range(-1, NUN + 1):
        for t in range(NT):
            stream += [(i, t, r) for r in range(128 - 16, VR - 1, -16)]
            pv_at[len(stream) + DLY] = (i, t)
    seq = []
    for n, e in enumerate(stream):
        if n in pv_at:
            seq.append(('P',) + pv_at[n])
        seq.append(('K',) + e)
    base = min(n for n, e in enumerate(seq) if e[0] == 'K' and e[1] == 0)
    period = min(n for n, e in enumerate(seq) if e[0] == 'K' and e[1] == NUN) - base
    w0, w1 = base + ROT, base + ROT + period
    assert all(e[1] >= 0 for e in seq[w0:w1]) and all(e[0] == 'K' for e in seq[w0:w1] if e[1] == NUN)
    cblk = [e for e in seq[base:w0] if e[0] == 'K']
    jobs = [(i, t, s_, lt) for i in range(NUN + 1) for t in range(NT) for lt in range(NL) for s_ in range(2)]
    assert len(jobs) == period // NUN * (NUN + 1)
    j0 = seq.index(('P', 0, 0)) - 7 - LEAD
    kitems = [(d, t) for d in range(DH) for t in range(NT)]
    qitems = [(j, lt, half) for j in range(NQ) for lt in range(NL) for half in range(2)]
    kdl, qdl = {}, {}
    for hh in range(2):
        start = max(w0, j0 + hh * period // 2 + 2)
        hi = j0 + (hh + 1) * period // 2 - KMARGIN
        lo = start + KSTART
        for n, it in enumerate(kitems):
            kdl.setdefault(lo + (n + 1) * (hi - lo) // len(kitems), []).append((hh, it))
        lo = start + QSTART
        for n, it in enumerate(qitems):
            qdl.setdefault(lo + QOFF + n * (hi - lo) // len(qitems), []).append((hh, it))
    return seq, w0, w1, cblk, jobs, j0, qitems, kdl, qdl


SEQ, W0, W1, CBLK, JOBS, J0, QITEMS, KDL, QDL = _schedule()
CBLK_IDX = {(e[2], e[3]): n for n, e in enumerate(CBLK)}
JIDX = {j: m for m, j in enumerate(JOBS)}
N_JOB = W1 - W0
N_CJOB = W0 + HEAD - J0


def _kernel(xa, wa, woa, xb, wb, wob, o_hbm,
            x_buf, w_buf, wo_buf, k_scr, vt_scr, qt_scr, qu_scr, qf_scr, ot_scr, kba, kbb, qba, qbb,
            cp_scr, cj_scr, qn_scr, km_scr, vm_scr, ku_scr, flag_ref,
            sem_x, sem_w, sem_wo, sem_o):
    xs, ws, wos = (xa, xb), (wa, wb), (woa, wob)
    o_buf = x_buf

    def x_copy(p, j):
        return pltpu.make_async_copy(
            xs[p].at[0, pl.ds(j * TQ, TQ), :], x_buf.at[p * NQ + j], sem_x.at[p * NQ + j])

    def x_wait(t):
        pltpu.make_async_copy(x_buf.at[t], x_buf.at[t], sem_x.at[t]).wait()

    def w_copy(p, c):
        return pltpu.make_async_copy(
            ws[p].at[:, pl.ds(c * D, D)], w_buf.at[p * 3 + c], sem_w.at[p * 3 + c])

    def wo_copy(p):
        return pltpu.make_async_copy(wos[p], wo_buf.at[p], sem_wo.at[p])

    def o_copy(t, s_):
        p, j = t // NQ, t % NQ
        return pltpu.make_async_copy(
            o_buf.at[t, pl.ds(s_ * TO, TO)],
            o_hbm.at[0, pl.ds(j * TQ + s_ * TO, TO), pl.ds(p * D, D)],
            sem_o.at[t * (TQ // TO) + s_])

    w_copy(0, 1).start()
    x_copy(0, 0).start()
    flag_ref[...] = jnp.ones(flag_ref.shape, jnp.int32)
    qn_scr[...] = jnp.zeros(qn_scr.shape, F32)
    km_scr[...] = jnp.zeros(km_scr.shape, F32)
    vm_scr[...] = jnp.zeros(vm_scr.shape, F32)

    def split(u):
        return pltpu.bitcast(u << 16, F32), pltpu.bitcast(u & jnp.uint32(0xFFFF0000), F32)

    tdims = (((0,), (1,)), ((), ()))

    def proj_k1(p, x):
        k = jnp.dot(x, w_buf[p * 3 + 1], preferred_element_type=F32)
        km_scr[...] = jnp.maximum(km_scr[...], jnp.max(jnp.abs(k).reshape(TQ // 8, 8, D), axis=0))
        kb16 = k.astype(BF16)
        ku = pltpu.bitcast(kb16, U32)
        kr = pltpu.bitcast(kb16.astype(F32), U32)
        return jnp.concatenate(
            [(kr[r:r + 8] >> 16) | kr[r + 8:r + 16] if r % 128 < VR else ku[r // 2:r // 2 + 8]
             for r in range(0, TQ, 16)], axis=0)

    def proj_k2(t, p, j, ku):
        if not (isinstance(t, int) and t >= NQ):
            for d in range(DH):
                for b in range(TQ // 128):
                    kba[t * (TQ // 128) + b, d] = jnp.stack(
                        split(jnp.broadcast_to(ku[b * 64:b * 64 + 8, d:d + 1], (8, 128))))
        r0 = j * (TQ // 2)
        if not isinstance(r0, int):
            r0 = pl.multiple_of(r0, TQ // 2)
        for g in range(4):
            kg = ku[:, g * 128:(g + 1) * 128]
            for jj in range(8):
                k_scr[p * H + g * 8 + jj, pl.ds(r0, TQ // 2), :] = (
                    kg if jj == 0 else pltpu.roll(kg, 128 - DH * jj, 1))

    def proj_q(t, p, x):
        qt = lax.dot_general(w_buf[p * 3], x, tdims, preferred_element_type=F32)
        qu_scr[t] = pltpu.bitcast(qt.astype(BF16), U32).reshape(H, 8, TQ)
        qb = (qt * (LOG2E * DH ** -0.5)).astype(BF16)
        qt_scr[t] = pltpu.bitcast(qb, U32).reshape(H, 8, TQ)
        qf = qb.astype(F32)
        qn_scr[...] = jnp.maximum(qn_scr[...], jnp.sum((qf * qf).reshape(H, DH, TQ), axis=1))
        for lt in range(NL):
            qf_scr[t, :, lt] = qf[:, lt * 128:(lt + 1) * 128].reshape(H, 2, 8, 128)

    def proj_v(t, p, x):
        vt = lax.dot_general(w_buf[p * 3 + 2], x, tdims, preferred_element_type=F32)
        vm_scr[...] = jnp.maximum(vm_scr[...], jnp.max(jnp.abs(vt).reshape(D // 8, 8, TQ), axis=0))
        vt_scr[t] = pltpu.bitcast(vt.astype(BF16), U32).reshape(H, 8, TQ)

    def proj(t):
        p, j = (t // NQ, t % NQ) if isinstance(t, int) else (lax.shift_right_logical(t, 2), t & (NQ - 1))
        x_wait(t)
        x = x_buf[t]
        proj_k2(t, p, j, proj_k1(p, x))
        proj_q(t, p, x)
        proj_v(t, p, x)

    def proj_step(t, carry):
        @pl.when(t == NQ)
        def _():
            for c in range(3):
                w_copy(1, c).wait()

        proj(t)
        return carry

    w_copy(0, 1).wait()
    x_copy(0, 0).wait()
    w_copy(0, 0).start()
    w_copy(0, 2).start()
    ku_scr[...] = proj_k1(0, x_buf[0])
    w_copy(0, 0).wait()
    w_copy(0, 2).wait()
    for j in range(1, NQ):
        x_copy(0, j).start()
    proj_k2(0, 0, 0, ku_scr[...])
    proj_q(0, 0, x_buf[0])
    proj_v(0, 0, x_buf[0])
    for c in range(3):
        w_copy(1, c).start()
    for j in range(NQ):
        x_copy(1, j).start()
    wo_copy(0).start()
    wo_copy(1).start()
    lax.fori_loop(1, 2 * NQ - 1, proj_step, 0)
    proj(2 * NQ - 1)

    z = jnp.max(km_scr[...], axis=0, keepdims=True)
    z = jnp.broadcast_to(z * z, (8, D))
    zs = []
    for g in range(4):
        zg = z[:, g * 128:(g + 1) * 128]
        for sh in (1, 2, 4, 8):
            zg = zg + pltpu.roll(zg, sh, 1)
        zs.append(zg)
    kn2 = jnp.max(jnp.maximum(jnp.maximum(zs[0], zs[1]), jnp.maximum(zs[2], zs[3])))
    qn2 = jnp.max(qn_scr[...])
    vmax = jnp.max(vm_scr[...])
    safe = jnp.logical_and(qn2 * kn2 * 1.05 <= SAFE_LOG2 * SAFE_LOG2,
                           jnp.logical_and(vmax >= 2.0 ** -20, vmax <= 2.0 ** 24))

    def unit(ph, j, odd):
        p = lax.shift_right_logical(ph, 5)
        return dict(ph=ph, p=p, h=ph & (H - 1), j=j, tq=p * NQ + j, kb=(kba, kbb)[odd], qb=(qba, qbb)[odd],
                    l8=None, acc=None, w=None)

    def kblk(u, t, r):
        row = (t * 128 + r) // 2
        return k_scr[u['ph'], row:row + 8, :]

    def bcast_k(u, d, t, pre):
        if ('src', t) not in u:
            u[('src', t)] = kblk(u, t, 0)
        lo, hi = split(jnp.broadcast_to(pre(u[('src', t)])[:, d:d + 1], (8, 128)))
        u['kb'][t, d] = jnp.stack([lo, hi])
        return lo

    def bcast_q(u, j, lt, half, pre):
        src = pre(qf_scr[u['p'] * NQ + j, u['h'], lt, half])
        vs = [jnp.broadcast_to(src[s_:s_ + 1, :], (8, 128)) for s_ in range(8)]
        u['qb'][j * NL + lt, half * 8:half * 8 + 8] = jnp.stack(vs)
        return vs[-1]

    def vjob(u, t, s_, lt):
        if ('k', t) not in u:
            u[('k', t)] = u['kb'][t]
        if ('q', lt) not in u:
            u[('q', lt)] = u['qb'][u['j'] * NL + lt]
        kv, qv = u[('k', t)][:, s_], u[('q', lt)]
        acc = kv[0:2] * qv[0:2]
        for d in range(2, DH, 2):
            acc = acc + kv[d:d + 2] * qv[d:d + 2]
        return acc[0] + acc[1]

    def qk(u, blks):
        if u['w'] is None:
            u['w'] = pltpu.bitcast(qt_scr[u['tq'], u['h']], BF16)
        kc = pltpu.bitcast(jnp.concatenate(blks, axis=0), BF16)[:, :DH]
        return jnp.dot(kc, u['w'], preferred_element_type=F32)

    def fast_step(jb, carry):
        flags = [flag_ref[k] > 0 for k in range(NFLAG)]

        def tie(x, dep, k=0):
            return jnp.where(flags[k], x, pltpu.bitcast(dep, x.dtype))

        units = [unit(jb * 2 + i // NQ, i % NQ, i // NQ) for i in range(NUN)]
        units.append(unit(jnp.minimum(jb * 2 + 2, 2 * H - 1), 0, 0))
        sval = {m: cj_scr[m] for m in range(N_CJOB)}
        rows, popped, extra = {}, {}, {}
        for (t, r), n in CBLK_IDX.items():
            fin = jnp.exp2 if n >= len(CBLK) - CRAW else (lambda v: v)
            rows[(0, t, r)] = fin(cp_scr[n * 16:n * 16 + 8, :])
            rows[(0, t, r + 8)] = fin(cp_scr[n * 16 + 8:n * 16 + 16, :])

        def run_job(m):
            sval[m] = vjob(units[JOBS[m][0]], *JOBS[m][1:])
            if JOBS[m][0] == NUN:
                cj_scr[m - N_JOB] = sval[m]
            return sval[m]

        def operand(x, pos):
            due = []
            for fn, table, lag in ((bcast_k, KDL, KSTART), (bcast_q, QDL, QSTART)):
                for hh, it in table.get(pos, []):
                    src = popped[max(k for k in popped if k <= pos - lag)]
                    due.append(fn(units[(hh + 1) * NQ], *it, lambda v: tie(v, src)))
            if pos >= W0 + HEAD:
                due.append(run_job(pos - J0))
            due += extra.pop(pos, [])
            for k, dep in enumerate(due):
                x = tie(x, dep, k)
            return x

        def pv(i, t, pos):
            u = units[i]
            for s_ in range(2):
                rows[(i, t, 8 * s_)] = jnp.exp2(
                    jnp.concatenate([sval[JIDX[(i, t, s_, lt)]] for lt in range(NL)], axis=1))
            for r in range(120, -1, -8):
                u['l8'] = rows[(i, t, r)] if u['l8'] is None else u['l8'] + rows[(i, t, r)]
            pt = jnp.concatenate([rows.pop((i, t, r)) for r in range(0, 128, 8)], axis=0)
            vt = vt_scr[u['p'] * NQ + t // NL, u['h'], :, (t % NL) * 128:(t % NL + 1) * 128]
            o = jnp.dot(pltpu.bitcast(operand(vt, pos), BF16), pt, preferred_element_type=F32)
            u['acc'] = o if u['acc'] is None else u['acc'] + o
            if t == 0:
                for n in range(NL):
                    extra.setdefault(pos + FIRST + n, []).append(o[0:8, n * 128:(n + 1) * 128])
            if t == NT - 1:
                l = jnp.sum(u['l8'], axis=0, keepdims=True)
                ot_scr[u['tq'], u['h']] = pltpu.bitcast((u['acc'] * (1.0 / l)).astype(BF16), U32)

        n = W0
        while n < W1:
            e = SEQ[n]
            if e[0] == 'P':
                pv(e[1], e[2], n)
                n += 1
                continue
            n1 = n
            while n1 < W1 and SEQ[n1][0] == 'K' and SEQ[n1][1] == e[1]:
                n1 += 1
            u = units[e[1]]
            blk = {}
            for t in sorted({SEQ[k][2] for k in range(n, n1)}):
                rs = [SEQ[k][3] for k in range(n, n1) if SEQ[k][2] == t]
                run = k_scr[u['ph'], (t * 128 + min(rs)) // 2:(t * 128 + max(rs)) // 2 + 8, :]
                for r in rs:
                    blk[(t, r)] = run[(r - min(rs)) // 2:(r - min(rs)) // 2 + 8]
            st = qk(u, [operand(blk[SEQ[k][2:]], k) for k in range(n, n1)])
            pm = jnp.exp2(st)
            for bi, k in enumerate(range(n, n1)):
                _, i, t, r = SEQ[k]
                if i == NUN:
                    c = CBLK_IDX[(t, r)]
                    cp_scr[c * 16:c * 16 + 16, :] = (st if c >= len(CBLK) - CRAW else pm)[bi * 16:bi * 16 + 16]
                else:
                    rows[(i, t, r)] = pm[bi * 16:bi * 16 + 8]
                    rows[(i, t, r + 8)] = pm[bi * 16 + 8:bi * 16 + 16]
                popped[k] = st[bi * 16:bi * 16 + 8, 0:128]
            n = n1
        for m in range(W1 - J0, N_JOB + N_CJOB):
            run_job(m)
        return carry

    def slow_step(n, carry):
        u = unit(lax.shift_right_logical(n, 2), n & (NQ - 1), 0)
        w = pltpu.bitcast(qu_scr[u['tq'], u['h']], BF16)

        def scores(c):
            ku = k_scr[u['ph'], pl.ds(pl.multiple_of(c * (TQ // 2), TQ // 2), TQ // 2), :]
            blks = [ku[r // 2:r // 2 + 8] for r in range(0, TQ, 16)]
            for b in range(0, TQ // 16, 8):
                blks[b] = pltpu.bitcast(jnp.concatenate(split(blks[b]), axis=0).astype(BF16), U32)
            kc = pltpu.bitcast(jnp.concatenate(blks, axis=0), BF16)[:, :DH]
            s = jnp.dot(kc, w, preferred_element_type=F32)
            return s.astype(BF16).astype(F32) * DH ** -0.5

        m = lax.fori_loop(0, NQ, lambda c, m: jnp.maximum(m, jnp.max(scores(c), axis=0, keepdims=True)),
                          jnp.full((1, TQ), -jnp.inf, F32))

        def chunk(c, st):
            pt = jnp.exp((scores(c) - m).astype(BF16).astype(F32)).astype(BF16)
            vt = pltpu.bitcast(vt_scr[u['p'] * NQ + c, u['h']], BF16)
            return (st[0] + jnp.sum(pt.astype(F32), axis=0, keepdims=True),
                    st[1] + jnp.dot(vt, pt, preferred_element_type=F32))

        l, acc = lax.fori_loop(0, NQ, chunk, (jnp.zeros((1, TQ), F32), jnp.zeros((DH, TQ), F32)))
        ot_scr[u['tq'], u['h']] = pltpu.bitcast((acc / l).astype(BF16), U32)
        return carry

    u0 = unit(jnp.int32(0), 0, 0)
    for it in QITEMS:
        bcast_q(u0, *it, lambda v: v)
    st0 = qk(u0, [kblk(u0, e[2], e[3]) for e in CBLK])
    ne = (len(CBLK) - CRAW) * 16
    cp_scr[0:ne, :] = jnp.exp2(st0[0:ne])
    cp_scr[ne:, :] = st0[ne:]
    for m in range(N_CJOB):
        cj_scr[m] = vjob(u0, *JOBS[m][1:])

    @pl.when(safe)
    def _():
        lax.fori_loop(0, H, fast_step, 0)

    @pl.when(jnp.logical_not(safe))
    def _():
        lax.fori_loop(0, 2 * H * NQ, slow_step, 0)

    wo_copy(0).wait()
    wo_copy(1).wait()
    for t in range(2 * NQ):
        for s_ in range(TQ // TO):
            o_t = pltpu.bitcast(ot_scr[t, :, :, s_ * TO:(s_ + 1) * TO].reshape(H * 8, TO), BF16)
            out = lax.dot_general(o_t, wo_buf[t // NQ], (((0,), (0,)), ((), ())), preferred_element_type=F32)
            o_buf[t, s_ * TO:(s_ + 1) * TO, :] = out.astype(BF16)
            o_copy(t, s_).start()
    for t in range(2 * NQ):
        for s_ in range(TQ // TO):
            o_copy(t, s_).wait()


@jax.jit
def pallas_concat_heads__softmax_full_mha__softmax_full_mha__prompt_kernel(
    A_x: jax.Array,
    A_wqkv: jax.Array,
    A_wo: jax.Array,
    B_x: jax.Array,
    B_wqkv: jax.Array,
    B_wo: jax.Array,
):
    anyspec = pl.BlockSpec(memory_space=pl.ANY)
    return pl.pallas_call(
        _kernel,
        in_specs=[anyspec] * 6,
        out_specs=anyspec,
        out_shape=jax.ShapeDtypeStruct((1, S, 2 * D), BF16),
        scratch_shapes=[
            pltpu.VMEM((2 * NQ, TQ, D), BF16),
            pltpu.VMEM((6, D, D), BF16),
            pltpu.VMEM((2, D, D), BF16),
            pltpu.VMEM((2 * H, S // 2, 128), U32),
            pltpu.VMEM((2 * NQ, H, 8, TQ), U32),
            pltpu.VMEM((2 * NQ, H, 8, TQ), U32),
            pltpu.VMEM((2 * NQ, H, 8, TQ), U32),
            pltpu.VMEM((2 * NQ, H, NL, 2, 8, 128), F32),
            pltpu.VMEM((2 * NQ, H, 8, TQ), U32),
            pltpu.VMEM((2 * NT, DH, 2, 8, 128), F32),
            pltpu.VMEM((NT, DH, 2, 8, 128), F32),
            pltpu.VMEM((NQ * NL, DH, 8, 128), F32),
            pltpu.VMEM((NQ * NL, DH, 8, 128), F32),
            pltpu.VMEM((len(CBLK) * 16, TQ), F32),
            pltpu.VMEM((N_CJOB, 8, 128), F32),
            pltpu.VMEM((H, TQ), F32),
            pltpu.VMEM((8, D), F32),
            pltpu.VMEM((8, TQ), F32),
            pltpu.VMEM((TQ // 2, D), U32),
            pltpu.VMEM((NFLAG, 8, 128), jnp.int32),
            pltpu.SemaphoreType.DMA((2 * NQ,)),
            pltpu.SemaphoreType.DMA((6,)),
            pltpu.SemaphoreType.DMA((2,)),
            pltpu.SemaphoreType.DMA((2 * NQ * (TQ // TO),)),
        ],
        compiler_params=pltpu.CompilerParams(vmem_limit_bytes=96 * 1024 * 1024),
    )(A_x, A_wqkv, A_wo, B_x, B_wqkv, B_wo)
```

```python
import math

import jax
import jax.numpy as jnp
from jax import lax
import jax.experimental.pallas as pl
import jax.experimental.pallas.tpu as pltpu

S, D, H, DH = 2048, 512, 32, 16
LOG2E = math.log2(math.e)
F32, BF16, U32 = jnp.float32, jnp.bfloat16, jnp.uint32
TQ = 512
NQ = S // TQ
NT = S // 128
NL = TQ // 128
NUN = 2 * NQ
VROWS = [32 if t in (4, 12) else 16 for t in range(NT)]
TO = 128
NFLAG = 5
SAFE_LOG2 = 80.0

VBLK = [(t, r) for t in range(NT) for r in range(0, VROWS[t], 16)]
VREL = sorted({(t * 128 + r) % TQ for t, r in VBLK})
VMASK = {o: sum(1 << c for c in range(NQ) if ((c * TQ + o) // 128, o % 128) in VBLK) for o in VREL}
KSLOT = {(t, r): (t * 128 // TQ) * len(VREL) + VREL.index((t * 128 + r) % TQ) for t, r in VBLK}

DLY, LEAD, ROT, HEAD, FIRST, CRAW, XLAG = 8, 18, 14, 3, 8, 1, 3
KSTART, QSTART, QOFF, KMARGIN = 19, 13, 3, 3


def _schedule():
    stream, pv_at = [], {}
    for i in range(-1, NUN + 1):
        for t in range(NT):
            stream += [(i, t, r) for r in range(128 - 16, VROWS[t] - 1, -16)]
            pv_at[len(stream) + DLY] = (i, t)
    seq = []
    for n, e in enumerate(stream):
        if n in pv_at:
            seq.append(('P',) + pv_at[n])
        seq.append(('K',) + e)
    base = min(n for n, e in enumerate(seq) if e[0] == 'K' and e[1] == 0)
    period = min(n for n, e in enumerate(seq) if e[0] == 'K' and e[1] == NUN) - base
    w0, w1 = base + ROT, base + ROT + period
    assert all(e[1] >= 0 for e in seq[w0:w1]) and all(e[0] == 'K' for e in seq[w0:w1] if e[1] == NUN)
    cblk = [e for e in seq[base:w0] if e[0] == 'K']
    jobs = [(i, t, r, lt) for i in range(NUN + 1) for t in range(NT) for lt in range(NL)
            for r in range(0, VROWS[t], 8)]
    n_job = len(jobs) // (NUN + 1) * NUN
    j0 = seq.index(('P', 0, 0)) - 8 - LEAD
    due = [j0 + ((m + 1) * period) // n_job for m in range(len(jobs))]
    n_cjob = sum(1 for d in due if d < w0 + HEAD)
    n_in, n_x = n_job - HEAD, n_job - period
    xk = {((e + 1) * n_in) // n_x - 1 for e in range(n_x)}
    jat, xat, pos = {}, {}, w0 + HEAD
    for k in range(n_in):
        m = n_cjob + k
        due[m] = min(pos, w1 - 1)
        if k in xk:
            xat[due[m]] = m
        else:
            jat[pos] = m
            pos += 1
        assert jobs[m][0] == NUN or due[m] + XLAG <= seq.index(('P',) + jobs[m][:2]) - 3
    kitems = [(d, b) for d in range(DH) for b in VBLK]
    qitems = [(j, lt, half) for j in range(NQ) for lt in range(NL) for half in range(2)]
    kdl, qdl = {}, {}
    for hh in range(2):
        start = max(w0, due[hh * n_job // 2] + 2)
        hi = due[(hh + 1) * n_job // 2] - KMARGIN
        lo = start + KSTART
        for n, it in enumerate(kitems):
            kdl.setdefault(lo + (n + 1) * (hi - lo) // len(kitems), []).append((hh, it))
        lo = start + QSTART
        for n, it in enumerate(qitems):
            qdl.setdefault(lo + QOFF + n * (hi - lo) // len(qitems), []).append((hh, it))
    return seq, w0, w1, cblk, jobs, n_job, n_cjob, jat, xat, kdl, qdl


SEQ, W0, W1, CBLK, JOBS, N_JOB, N_CJOB, JAT, XAT, KDL, QDL = _schedule()
CBLK_IDX = {(e[2], e[3]): n for n, e in enumerate(CBLK)}
JIDX = {j: m for m, j in enumerate(JOBS)}


def _kernel(xa, wa, woa, xb, wb, wob, o_hbm,
            x_buf, w_buf, wo_buf, k_scr, vt_scr, qt_scr, qu_scr, qf_scr, ot_scr, kba, kbb, qba, qbb,
            cp_scr, cj_scr, qn_scr, km_scr, vm_scr, flag_ref,
            sem_x, sem_w, sem_wo, sem_o):
    xs, ws, wos = (xa, xb), (wa, wb), (woa, wob)
    o_buf = x_buf

    def x_copy(p, j):
        return pltpu.make_async_copy(
            xs[p].at[0, pl.ds(j * TQ, TQ), :], x_buf.at[p * NQ + j], sem_x.at[p * NQ + j])

    def x_wait(t):
        pltpu.make_async_copy(x_buf.at[t], x_buf.at[t], sem_x.at[t]).wait()

    def w_copy(p, c):
        return pltpu.make_async_copy(
            ws[p].at[:, pl.ds(c * D, D)], w_buf.at[p * 3 + c], sem_w.at[p * 3 + c])

    def wo_copy(p):
        return pltpu.make_async_copy(wos[p], wo_buf.at[p], sem_wo.at[p])

    def o_copy(t, s_):
        p, j = t // NQ, t % NQ
        return pltpu.make_async_copy(
            o_buf.at[t, pl.ds(s_ * TO, TO)],
            o_hbm.at[0, pl.ds(j * TQ + s_ * TO, TO), pl.ds(p * D, D)],
            sem_o.at[t * (TQ // TO) + s_])

    w_copy(0, 0).start()
    x_copy(0, 0).start()
    flag_ref[...] = jnp.ones(flag_ref.shape, jnp.int32)
    qn_scr[...] = jnp.zeros(qn_scr.shape, F32)
    km_scr[...] = jnp.zeros(km_scr.shape, F32)
    vm_scr[...] = jnp.zeros(vm_scr.shape, F32)

    def pick(o, c, vpu_form, mxu_form):
        mask = VMASK.get(o, 0)
        if isinstance(c, int) or mask in (0, (1 << NQ) - 1):
            return vpu_form() if (mask >> (c if isinstance(c, int) else 0)) & 1 else mxu_form
        return jnp.where((lax.shift_right_logical(mask, c) & 1) == 1, vpu_form(), mxu_form)

    def split(u):
        return pltpu.bitcast(u << 16, F32), pltpu.bitcast(u & jnp.uint32(0xFFFF0000), F32)

    tdims = (((0,), (1,)), ((), ()))

    def proj_k(t, p, j, x):
        k = jnp.dot(x, w_buf[p * 3 + 1], preferred_element_type=F32)
        km_scr[...] = jnp.maximum(km_scr[...], jnp.max(jnp.abs(k).reshape(TQ // 8, 8, D), axis=0))
        kb16 = k.astype(BF16)
        ku = pltpu.bitcast(kb16, U32)
        kr = pltpu.bitcast(kb16.astype(F32), U32)
        ku = jnp.concatenate(
            [pick(r, j, lambda r=r: (kr[r:r + 8] >> 16) | kr[r + 8:r + 16], ku[r // 2:r // 2 + 8])
             for r in range(0, TQ, 16)], axis=0)
        if not (isinstance(t, int) and t >= NQ):
            for d in range(DH):
                for b, o in enumerate(VREL):
                    kba[t * len(VREL) + b, d] = jnp.stack(
                        split(jnp.broadcast_to(ku[o // 2:o // 2 + 8, d:d + 1], (8, 128))))
        r0 = j * (TQ // 2)
        if not isinstance(r0, int):
            r0 = pl.multiple_of(r0, TQ // 2)
        for g in range(4):
            kg = ku[:, g * 128:(g + 1) * 128]
            for jj in range(8):
                k_scr[p * H + g * 8 + jj, pl.ds(r0, TQ // 2), :] = (
                    kg if jj == 0 else pltpu.roll(kg, 128 - DH * jj, 1))
        return ku

    def proj_q(t, p, x):
        qt = lax.dot_general(w_buf[p * 3], x, tdims, preferred_element_type=F32)
        qu_scr[t] = pltpu.bitcast(qt.astype(BF16), U32).reshape(H, 8, TQ)
        qb = (qt * (LOG2E * DH ** -0.5)).astype(BF16)
        qt_scr[t] = pltpu.bitcast(qb, U32).reshape(H, 8, TQ)
        qf = qb.astype(F32)
        qn_scr[...] = jnp.maximum(qn_scr[...], jnp.sum((qf * qf).reshape(H, DH, TQ), axis=1))
        for lt in range(NL):
            qf_scr[t, :, lt] = qf[:, lt * 128:(lt + 1) * 128].reshape(H, 2, 8, 128)
            if not (isinstance(t, int) and t >= NQ):
                qba[t * NL + lt] = jnp.stack(
                    [jnp.broadcast_to(qf[d:d + 1, lt * 128:(lt + 1) * 128], (8, 128)) for d in range(DH)])

    def proj_v(t, p, x):
        vt = lax.dot_general(w_buf[p * 3 + 2], x, tdims, preferred_element_type=F32)
        vm_scr[p] = jnp.maximum(vm_scr[p], jnp.max(jnp.abs(vt).reshape(D // 8, 8, TQ), axis=0))
        vt_scr[t] = pltpu.bitcast(vt.astype(BF16), U32).reshape(H, 8, TQ)

    def proj(t):
        p, j = (t // NQ, t % NQ) if isinstance(t, int) else (lax.shift_right_logical(t, 2), t & (NQ - 1))
        x_wait(t)
        x = x_buf[t]
        ku = proj_k(t, p, j, x)
        proj_q(t, p, x)
        proj_v(t, p, x)
        return ku

    def proj_step(t, carry):
        @pl.when(t == NQ)
        def _():
            for c in range(3):
                w_copy(1, c).wait()

        proj(t)
        return carry

    w_copy(0, 0).wait()
    x_copy(0, 0).wait()
    w_copy(0, 1).start()
    w_copy(0, 2).start()
    proj_q(0, 0, x_buf[0])
    w_copy(0, 1).wait()
    w_copy(0, 2).wait()
    for j in range(1, NQ):
        x_copy(0, j).start()
    proj_k(0, 0, 0, x_buf[0])
    proj_v(0, 0, x_buf[0])
    for c in range(3):
        w_copy(1, c).start()
    for j in range(NQ):
        x_copy(1, j).start()
    wo_copy(0).start()
    wo_copy(1).start()
    lax.fori_loop(1, 2 * NQ - 1, proj_step, 0)
    ku_last = proj(2 * NQ - 1)

    z = jnp.max(km_scr[...], axis=0, keepdims=True)
    z = jnp.broadcast_to(z * z, (8, D))
    zs = []
    for g in range(4):
        zg = z[:, g * 128:(g + 1) * 128]
        for sh in (1, 2, 4, 8):
            zg = zg + pltpu.roll(zg, sh, 1)
        zs.append(zg)
    kn2 = jnp.max(jnp.maximum(jnp.maximum(zs[0], zs[1]), jnp.maximum(zs[2], zs[3])))
    qn2 = jnp.max(qn_scr[...])
    safe = qn2 * kn2 * 1.05 <= SAFE_LOG2 * SAFE_LOG2
    for p in range(2):
        vmax = jnp.max(vm_scr[p])
        safe = jnp.logical_and(safe, jnp.logical_and(vmax >= 2.0 ** -20, vmax <= 2.0 ** 24))

    def unit(ph, j, odd):
        p = lax.shift_right_logical(ph, 5)
        return dict(ph=ph, p=p, h=ph & (H - 1), j=j, tq=p * NQ + j, kb=(kba, kbb)[odd], qb=(qba, qbb)[odd],
                    l8=None, acc=None, w=None)

    def kblk(u, t, r):
        row = (t * 128 + r) // 2
        return k_scr[u['ph'], row:row + 8, :]

    def bcast_k(u, d, b, pre):
        if ('src', b) not in u:
            u[('src', b)] = kblk(u, *b)
        lo, hi = split(jnp.broadcast_to(pre(u[('src', b)])[:, d:d + 1], (8, 128)))
        u['kb'][KSLOT[b], d] = jnp.stack([lo, hi])
        return lo

    def bcast_q(u, j, lt, half, pre):
        src = pre(qf_scr[u['p'] * NQ + j, u['h'], lt, half])
        vs = [jnp.broadcast_to(src[s_:s_ + 1, :], (8, 128)) for s_ in range(8)]
        u['qb'][j * NL + lt, half * 8:half * 8 + 8] = jnp.stack(vs)
        return vs[-1]

    def vjob(u, t, r, lt, pre=None, first=None):
        b, jl = (t, r // 16 * 16), u['j'] * NL + lt
        if pre is not None:
            kv, qv = pre(u['kb'][KSLOT[b], :, r // 8 % 2]), u['qb'][jl]
        else:
            if ('k', b) not in u:
                u[('k', b)] = u['kb'][KSLOT[b]]
            if ('q', lt) not in u:
                u[('q', lt)] = u['qb'][jl]
            kv, qv = u[('k', b)][:, r // 8 % 2], u[('q', lt)]
        w = 2 if first is None else 1
        acc = kv[0:w] * qv[0:w]
        if first is not None:
            acc = first(acc[0])[None]
        for d in range(w, DH, w):
            acc = acc + kv[d:d + w] * qv[d:d + w]
        return acc[0] + acc[1] if w == 2 else acc[0]

    def qk(u, blks):
        if u['w'] is None:
            u['w'] = pltpu.bitcast(qt_scr[u['tq'], u['h']], BF16)
        kc = pltpu.bitcast(jnp.concatenate(blks, axis=0), BF16)[:, :DH]
        return jnp.dot(kc, u['w'], preferred_element_type=F32)

    def fast_step(jb, carry):
        flags = [flag_ref[k] > 0 for k in range(NFLAG)]

        def tie(x, dep, k=0):
            return jnp.where(flags[k], x, pltpu.bitcast(dep, x.dtype))

        units = [unit(jb * 2 + i // NQ, i % NQ, i // NQ) for i in range(NUN)]
        units.append(unit(jnp.minimum(jb * 2 + 2, 2 * H - 1), 0, 0))
        sval = {m: cj_scr[m] for m in range(N_CJOB)}
        rows, popped, extra = {}, {}, {}
        for (t, r), n in CBLK_IDX.items():
            fin = jnp.exp2 if n >= len(CBLK) - CRAW else (lambda v: v)
            rows[(0, t, r)] = fin(cp_scr[n * 16:n * 16 + 8, :])
            rows[(0, t, r + 8)] = fin(cp_scr[n * 16 + 8:n * 16 + 16, :])

        chain = []

        def run_job(m, first=None):
            sval[m] = vjob(units[JOBS[m][0]], *JOBS[m][1:], first=first)
            if JOBS[m][0] == NUN:
                cj_scr[m - N_JOB] = sval[m]
            return sval[m]

        def operand(x, pos):
            due = []
            for fn, table, lag in ((bcast_k, KDL, KSTART), (bcast_q, QDL, QSTART)):
                for hh, it in table.get(pos, []):
                    src = popped[max(k for k in popped if k <= pos - lag)]
                    due.append(fn(units[(hh + 1) * NQ], *it, lambda v: tie(v, src)))
            if pos in XAT:
                chain.append(run_job(XAT[pos], lambda v: tie(v, chain[-1]) if chain else v))
                if pos + XLAG < W1:
                    extra.setdefault(pos + XLAG, []).append(chain[-1])
            if pos in JAT:
                due.append(run_job(JAT[pos]))
            due += extra.pop(pos, [])
            for k, dep in enumerate(due):
                x = tie(x, dep, k)
            return x

        def pv(i, t, pos):
            u = units[i]
            for r in range(0, VROWS[t], 8):
                rows[(i, t, r)] = jnp.exp2(
                    jnp.concatenate([sval[JIDX[(i, t, r, lt)]] for lt in range(NL)], axis=1))
            for r in range(120, -1, -8):
                u['l8'] = rows[(i, t, r)] if u['l8'] is None else u['l8'] + rows[(i, t, r)]
            pt = jnp.concatenate([rows.pop((i, t, r)) for r in range(0, 128, 8)], axis=0)
            vt = vt_scr[u['p'] * NQ + t // NL, u['h'], :, (t % NL) * 128:(t % NL + 1) * 128]
            o = jnp.dot(pltpu.bitcast(operand(vt, pos), BF16), pt, preferred_element_type=F32)
            u['acc'] = o if u['acc'] is None else u['acc'] + o
            if t == 0:
                for n in range(NL):
                    extra.setdefault(pos + FIRST + n, []).append(o[0:8, n * 128:(n + 1) * 128])
            if t == NT - 1:
                l = jnp.sum(u['l8'], axis=0, keepdims=True)
                r0 = pl.reciprocal(l, approx=True)
                r1 = r0 * (2.0 - l * r0)
                ot_scr[u['tq'], u['h']] = pltpu.bitcast((u['acc'] * r1).astype(BF16), U32)

        n = W0
        while n < W1:
            e = SEQ[n]
            if e[0] == 'P':
                pv(e[1], e[2], n)
                n += 1
                continue
            n1 = n
            while n1 < W1 and SEQ[n1][0] == 'K' and SEQ[n1][1] == e[1]:
                n1 += 1
            u = units[e[1]]
            blk = {}
            for t in sorted({SEQ[k][2] for k in range(n, n1)}):
                rs = [SEQ[k][3] for k in range(n, n1) if SEQ[k][2] == t]
                run = k_scr[u['ph'], (t * 128 + min(rs)) // 2:(t * 128 + max(rs)) // 2 + 8, :]
                for r in rs:
                    blk[(t, r)] = run[(r - min(rs)) // 2:(r - min(rs)) // 2 + 8]
            st = qk(u, [operand(blk[SEQ[k][2:]], k) for k in range(n, n1)])
            pm = jnp.exp2(st)
            for bi, k in enumerate(range(n, n1)):
                _, i, t, r = SEQ[k]
                if i == NUN:
                    c = CBLK_IDX[(t, r)]
                    cp_scr[c * 16:c * 16 + 16, :] = (st if c >= len(CBLK) - CRAW else pm)[bi * 16:bi * 16 + 16]
                else:
                    rows[(i, t, r)] = pm[bi * 16:bi * 16 + 8]
                    rows[(i, t, r + 8)] = pm[bi * 16 + 8:bi * 16 + 16]
                popped[k] = st[bi * 16:bi * 16 + 8, 0:128]
            n = n1
        for m in range(N_CJOB + N_JOB - HEAD, N_CJOB + N_JOB):
            run_job(m)
        return carry

    def slow_step(n, carry):
        u = unit(lax.shift_right_logical(n, 2), n & (NQ - 1), 0)
        w = pltpu.bitcast(qu_scr[u['tq'], u['h']], BF16)

        def scores(c):
            ku = k_scr[u['ph'], pl.ds(pl.multiple_of(c * (TQ // 2), TQ // 2), TQ // 2), :]
            blks = [ku[r // 2:r // 2 + 8] for r in range(0, TQ, 16)]
            blks = [pick(b * 16, c, lambda v=v: pltpu.bitcast(
                jnp.concatenate(split(v), axis=0).astype(BF16), U32), v) for b, v in enumerate(blks)]
            kc = pltpu.bitcast(jnp.concatenate(blks, axis=0), BF16)[:, :DH]
            s = jnp.dot(kc, w, preferred_element_type=F32)
            return s.astype(BF16).astype(F32) * DH ** -0.5

        m = lax.fori_loop(0, NQ, lambda c, m: jnp.maximum(m, jnp.max(scores(c), axis=0, keepdims=True)),
                          jnp.full((1, TQ), -jnp.inf, F32))

        def chunk(c, st):
            pt = jnp.exp((scores(c) - m).astype(BF16).astype(F32)).astype(BF16)
            vt = pltpu.bitcast(vt_scr[u['p'] * NQ + c, u['h']], BF16)
            return (st[0] + jnp.sum(pt.astype(F32), axis=0, keepdims=True),
                    st[1] + jnp.dot(vt, pt, preferred_element_type=F32))

        l, acc = lax.fori_loop(0, NQ, chunk, (jnp.zeros((1, TQ), F32), jnp.zeros((DH, TQ), F32)))
        ot_scr[u['tq'], u['h']] = pltpu.bitcast((acc / l).astype(BF16), U32)
        return carry

    u0 = unit(jnp.int32(0), 0, 0)
    st0 = qk(u0, [kblk(u0, e[2], e[3]) for e in CBLK])
    ne = (len(CBLK) - CRAW) * 16
    cp_scr[0:ne, :] = jnp.exp2(st0[0:ne])
    cp_scr[ne:, :] = st0[ne:]
    prev = pltpu.bitcast(ku_last[0:8, 0:128], F32)
    for m in range(N_CJOB):
        prev = vjob(u0, *JOBS[m][1:], pre=lambda v: jnp.where((flag_ref[0] > 0)[None], v, prev[None]))
        cj_scr[m] = prev

    @pl.when(safe)
    def _():
        lax.fori_loop(0, H, fast_step, 0)

    @pl.when(jnp.logical_not(safe))
    def _():
        lax.fori_loop(0, 2 * H * NQ, slow_step, 0)

    wo_copy(0).wait()
    wo_copy(1).wait()
    for t in range(2 * NQ):
        for s_ in range(TQ // TO):
            o_t = pltpu.bitcast(ot_scr[t, :, :, s_ * TO:(s_ + 1) * TO].reshape(H * 8, TO), BF16)
            out = lax.dot_general(o_t, wo_buf[t // NQ], (((0,), (0,)), ((), ())), preferred_element_type=F32)
            o_buf[t, s_ * TO:(s_ + 1) * TO, :] = out.astype(BF16)
            o_copy(t, s_).start()
    for t in range(2 * NQ):
        for s_ in range(TQ // TO):
            o_copy(t, s_).wait()


@jax.jit
def pallas_concat_heads__softmax_full_mha__softmax_full_mha__prompt_kernel(
    A_x: jax.Array,
    A_wqkv: jax.Array,
    A_wo: jax.Array,
    B_x: jax.Array,
    B_wqkv: jax.Array,
    B_wo: jax.Array,
):
    anyspec = pl.BlockSpec(memory_space=pl.ANY)
    return pl.pallas_call(
        _kernel,
        in_specs=[anyspec] * 6,
        out_specs=anyspec,
        out_shape=jax.ShapeDtypeStruct((1, S, 2 * D), BF16),
        scratch_shapes=[
            pltpu.VMEM((2 * NQ, TQ, D), BF16),
            pltpu.VMEM((6, D, D), BF16),
            pltpu.VMEM((2, D, D), BF16),
            pltpu.VMEM((2 * H, S // 2, 128), U32),
            pltpu.VMEM((2 * NQ, H, 8, TQ), U32),
            pltpu.VMEM((2 * NQ, H, 8, TQ), U32),
            pltpu.VMEM((2 * NQ, H, 8, TQ), U32),
            pltpu.VMEM((2 * NQ, H, NL, 2, 8, 128), F32),
            pltpu.VMEM((2 * NQ, H, 8, TQ), U32),
            pltpu.VMEM((2 * NQ * len(VREL), DH, 2, 8, 128), F32),
            pltpu.VMEM((NQ * len(VREL), DH, 2, 8, 128), F32),
            pltpu.VMEM((2 * NQ * NL, DH, 8, 128), F32),
            pltpu.VMEM((NQ * NL, DH, 8, 128), F32),
            pltpu.VMEM((len(CBLK) * 16, TQ), F32),
            pltpu.VMEM((N_CJOB, 8, 128), F32),
            pltpu.VMEM((H, TQ), F32),
            pltpu.VMEM((8, D), F32),
            pltpu.VMEM((2, 8, TQ), F32),
            pltpu.VMEM((NFLAG, 8, 128), jnp.int32),
            pltpu.SemaphoreType.DMA((2 * NQ,)),
            pltpu.SemaphoreType.DMA((6,)),
            pltpu.SemaphoreType.DMA((2,)),
            pltpu.SemaphoreType.DMA((2 * NQ * (TQ // TO),)),
        ],
        compiler_params=pltpu.CompilerParams(vmem_limit_bytes=96 * 1024 * 1024),
    )(A_x, A_wqkv, A_wo, B_x, B_wqkv, B_wo)
```

```python
import math

import jax
import jax.numpy as jnp
from jax import lax
import jax.experimental.pallas as pl
import jax.experimental.pallas.tpu as pltpu

S, D, H, DH = 2048, 512, 32, 16
LOG2E = math.log2(math.e)
F32, BF16, U32 = jnp.float32, jnp.bfloat16, jnp.uint32
TQ = 512
NQ = S // TQ
NT = S // 128
NL = TQ // 128
NUN = 2 * NQ
VROWS = [32 if t in (4, 12) else 16 for t in range(NT)]
TO = 128
NFLAG = 5
SAFE_LOG2 = 80.0

VBLK = [(t, r) for t in range(NT) for r in range(0, VROWS[t], 16)]
VREL = sorted({(t * 128 + r) % TQ for t, r in VBLK})
VMASK = {o: sum(1 << c for c in range(NQ) if ((c * TQ + o) // 128, o % 128) in VBLK) for o in VREL}
KSLOT = {(t, r): (t * 128 // TQ) * len(VREL) + VREL.index((t * 128 + r) % TQ) for t, r in VBLK}

DLY, LEAD, ROT, HEAD, FIRST, CRAW, XLAG = 8, 18, 14, 3, 8, 1, 3
KSTART, QSTART, QOFF, KMARGIN = 19, 13, 3, 3


def _schedule():
    stream, pv_at = [], {}
    for i in range(-1, NUN + 1):
        for t in range(NT):
            stream += [(i, t, r) for r in range(128 - 16, VROWS[t] - 1, -16)]
            pv_at[len(stream) + DLY] = (i, t)
    seq = []
    for n, e in enumerate(stream):
        if n in pv_at:
            seq.append(('P',) + pv_at[n])
        seq.append(('K',) + e)
    base = min(n for n, e in enumerate(seq) if e[0] == 'K' and e[1] == 0)
    period = min(n for n, e in enumerate(seq) if e[0] == 'K' and e[1] == NUN) - base
    w0, w1 = base + ROT, base + ROT + period
    assert all(e[1] >= 0 for e in seq[w0:w1]) and all(e[0] == 'K' for e in seq[w0:w1] if e[1] == NUN)
    cblk = [e for e in seq[base:w0] if e[0] == 'K']
    jobs = [(i, t, r, lt) for i in range(NUN + 1) for t in range(NT) for lt in range(NL)
            for r in range(0, VROWS[t], 8)]
    n_job = len(jobs) // (NUN + 1) * NUN
    j0 = seq.index(('P', 0, 0)) - 8 - LEAD
    due = [j0 + ((m + 1) * period) // n_job for m in range(len(jobs))]
    n_cjob = sum(1 for d in due if d < w0 + HEAD)
    n_in, n_x = n_job - HEAD, n_job - period
    xk = {((e + 1) * n_in) // n_x - 1 for e in range(n_x)}
    jat, xat, pos = {}, {}, w0 + HEAD
    for k in range(n_in):
        m = n_cjob + k
        due[m] = min(pos, w1 - 1)
        if k in xk:
            xat[due[m]] = m
        else:
            jat[pos] = m
            pos += 1
        assert jobs[m][0] == NUN or due[m] + XLAG <= seq.index(('P',) + jobs[m][:2]) - 3
    kitems = [(d, b) for d in range(DH) for b in VBLK]
    qitems = [(j, lt, half) for j in range(NQ) for lt in range(NL) for half in range(2)]
    kdl, qdl = {}, {}
    for hh in range(2):
        start = max(w0, due[hh * n_job // 2] + 2)
        hi = due[(hh + 1) * n_job // 2] - KMARGIN
        lo = start + KSTART
        for n, it in enumerate(kitems):
            kdl.setdefault(lo + (n + 1) * (hi - lo) // len(kitems), []).append((hh, it))
        lo = start + QSTART
        for n, it in enumerate(qitems):
            qdl.setdefault(lo + QOFF + n * (hi - lo) // len(qitems), []).append((hh, it))
    return seq, w0, w1, cblk, jobs, n_job, n_cjob, jat, xat, kdl, qdl


SEQ, W0, W1, CBLK, JOBS, N_JOB, N_CJOB, JAT, XAT, KDL, QDL = _schedule()
CBLK_IDX = {(e[2], e[3]): n for n, e in enumerate(CBLK)}
JIDX = {j: m for m, j in enumerate(JOBS)}


def _kernel(xa, wa, woa, xb, wb, wob, o_hbm,
            x_buf, w_buf, wo_buf, k_scr, vt_scr, qt_scr, qu_scr, qf_scr, ot_scr, kba, kbb, qba, qbb,
            cp_scr, cj_scr, qn_scr, km_scr, vm_scr, flag_ref,
            sem_x, sem_w, sem_wo, sem_o):
    xs, ws, wos = (xa, xb), (wa, wb), (woa, wob)
    o_buf = x_buf

    def x_copy(p, j):
        return pltpu.make_async_copy(
            xs[p].at[0, pl.ds(j * TQ, TQ), :], x_buf.at[p * NQ + j], sem_x.at[p * NQ + j])

    def x_wait(t):
        pltpu.make_async_copy(x_buf.at[t], x_buf.at[t], sem_x.at[t]).wait()

    def w_copy(p, c):
        return pltpu.make_async_copy(
            ws[p].at[:, pl.ds(c * D, D)], w_buf.at[p * 3 + c], sem_w.at[p * 3 + c])

    def wo_copy(p):
        return pltpu.make_async_copy(wos[p], wo_buf.at[p], sem_wo.at[p])

    def o_copy(t, s_):
        p, j = t // NQ, t % NQ
        return pltpu.make_async_copy(
            o_buf.at[t, pl.ds(s_ * TO, TO)],
            o_hbm.at[0, pl.ds(j * TQ + s_ * TO, TO), pl.ds(p * D, D)],
            sem_o.at[t * (TQ // TO) + s_])

    w_copy(0, 0).start()
    x_copy(0, 0).start()
    flag_ref[...] = jnp.ones(flag_ref.shape, jnp.int32)
    qn_scr[...] = jnp.zeros(qn_scr.shape, F32)
    km_scr[...] = jnp.zeros(km_scr.shape, F32)
    vm_scr[...] = jnp.zeros(vm_scr.shape, F32)

    def pick(o, c, vpu_form, mxu_form):
        mask = VMASK.get(o, 0)
        if isinstance(c, int) or mask in (0, (1 << NQ) - 1):
            return vpu_form() if (mask >> (c if isinstance(c, int) else 0)) & 1 else mxu_form
        return jnp.where((lax.shift_right_logical(mask, c) & 1) == 1, vpu_form(), mxu_form)

    def split(u):
        return pltpu.bitcast(u << 16, F32), pltpu.bitcast(u & jnp.uint32(0xFFFF0000), F32)

    tdims = (((0,), (1,)), ((), ()))

    def proj_k(t, p, j, x):
        k = jnp.dot(x, w_buf[p * 3 + 1], preferred_element_type=F32)
        km_scr[...] = jnp.maximum(km_scr[...], jnp.max(jnp.abs(k).reshape(TQ // 8, 8, D), axis=0))
        kb16 = k.astype(BF16)
        ku = pltpu.bitcast(kb16, U32)
        kr = pltpu.bitcast(kb16.astype(F32), U32)
        ku = jnp.concatenate(
            [pick(r, j, lambda r=r: (kr[r:r + 8] >> 16) | kr[r + 8:r + 16], ku[r // 2:r // 2 + 8])
             for r in range(0, TQ, 16)], axis=0)
        if not (isinstance(t, int) and t >= NQ):
            for d in range(DH):
                for b, o in enumerate(VREL):
                    kba[t * len(VREL) + b, d] = jnp.stack(
                        split(jnp.broadcast_to(ku[o // 2:o // 2 + 8, d:d + 1], (8, 128))))
        r0 = j * (TQ // 2)
        if not isinstance(r0, int):
            r0 = pl.multiple_of(r0, TQ // 2)
        for g in range(4):
            kg = ku[:, g * 128:(g + 1) * 128]
            for jj in range(8):
                k_scr[p * H + g * 8 + jj, pl.ds(r0, TQ // 2), :] = (
                    kg if jj == 0 else pltpu.roll(kg, 128 - DH * jj, 1))
        return ku

    def proj_q(t, p, x):
        qt = lax.dot_general(w_buf[p * 3], x, tdims, preferred_element_type=F32)
        qu_scr[t] = pltpu.bitcast(qt.astype(BF16), U32).reshape(H, 8, TQ)
        qb = (qt * (LOG2E * DH ** -0.5)).astype(BF16)
        qt_scr[t] = pltpu.bitcast(qb, U32).reshape(H, 8, TQ)
        qf = qb.astype(F32)
        qn_scr[...] = jnp.maximum(qn_scr[...], jnp.sum((qf * qf).reshape(H, DH, TQ), axis=1))
        for lt in range(NL):
            qf_scr[t, :, lt] = qf[:, lt * 128:(lt + 1) * 128].reshape(H, 2, 8, 128)
            if not (isinstance(t, int) and t >= NQ):
                qba[t * NL + lt] = jnp.stack(
                    [jnp.broadcast_to(qf[d:d + 1, lt * 128:(lt + 1) * 128], (8, 128)) for d in range(DH)])

    def proj_v(t, p, x):
        vt = lax.dot_general(w_buf[p * 3 + 2], x, tdims, preferred_element_type=F32)
        vm_scr[p] = jnp.maximum(vm_scr[p], jnp.max(jnp.abs(vt).reshape(D // 8, 8, TQ), axis=0))
        vt_scr[t] = pltpu.bitcast(vt.astype(BF16), U32).reshape(H, 8, TQ)

    def proj(t):
        p, j = (t // NQ, t % NQ) if isinstance(t, int) else (lax.shift_right_logical(t, 2), t & (NQ - 1))
        x_wait(t)
        x = x_buf[t]
        ku = proj_k(t, p, j, x)
        proj_q(t, p, x)
        proj_v(t, p, x)
        return ku

    def proj_step(t, carry):
        @pl.when(t == NQ)
        def _():
            for c in range(3):
                w_copy(1, c).wait()

        proj(t)
        return carry

    w_copy(0, 0).wait()
    x_copy(0, 0).wait()
    w_copy(0, 1).start()
    w_copy(0, 2).start()
    proj_q(0, 0, x_buf[0])
    w_copy(0, 1).wait()
    w_copy(0, 2).wait()
    for j in range(1, NQ):
        x_copy(0, j).start()
    proj_k(0, 0, 0, x_buf[0])
    proj_v(0, 0, x_buf[0])
    for c in range(3):
        w_copy(1, c).start()
    for j in range(NQ):
        x_copy(1, j).start()
    wo_copy(0).start()
    wo_copy(1).start()
    lax.fori_loop(1, 2 * NQ - 1, proj_step, 0)
    ku_last = proj(2 * NQ - 1)

    z = jnp.max(km_scr[...], axis=0, keepdims=True)
    z = jnp.broadcast_to(z * z, (8, D))
    zs = []
    for g in range(4):
        zg = z[:, g * 128:(g + 1) * 128]
        for sh in (1, 2, 4, 8):
            zg = zg + pltpu.roll(zg, sh, 1)
        zs.append(zg)
    kn2 = jnp.max(jnp.maximum(jnp.maximum(zs[0], zs[1]), jnp.maximum(zs[2], zs[3])))
    qn2 = jnp.max(qn_scr[...])
    safe = qn2 * kn2 * 1.05 <= SAFE_LOG2 * SAFE_LOG2
    for p in range(2):
        vmax = jnp.max(vm_scr[p])
        safe = jnp.logical_and(safe, jnp.logical_and(vmax >= 2.0 ** -20, vmax <= 2.0 ** 24))

    def unit(ph, j, odd):
        p = lax.shift_right_logical(ph, 5)
        return dict(ph=ph, p=p, h=ph & (H - 1), j=j, tq=p * NQ + j, kb=(kba, kbb)[odd], qb=(qba, qbb)[odd],
                    l8=None, acc=None, w=None)

    def cached(u, key, fn):
        if key not in u:
            u[key] = fn()
        return u[key]

    def kblk(u, t, r):
        row = (t * 128 + r) // 2
        return k_scr[u['ph'], row:row + 8, :]

    def bcast_k(u, d, b, pre):
        src = cached(u, ('src', b), lambda: kblk(u, *b))
        lo, hi = split(jnp.broadcast_to(pre(src)[:, d:d + 1], (8, 128)))
        u['kb'][KSLOT[b], d] = jnp.stack([lo, hi])
        return lo

    def bcast_q(u, j, lt, half, pre):
        src = pre(qf_scr[u['p'] * NQ + j, u['h'], lt, half])
        vs = [jnp.broadcast_to(src[s_:s_ + 1, :], (8, 128)) for s_ in range(8)]
        u['qb'][j * NL + lt, half * 8:half * 8 + 8] = jnp.stack(vs)
        return vs[-1]

    def vjob(u, t, r, lt, pre=None, first=None):
        b, half, jl = (t, r // 16 * 16), r // 8 % 2, u['j'] * NL + lt
        w = 2 if first is None else 1

        def pieces(v):
            return [v[d:d + w] for d in range(0, DH, w)]

        if pre is not None:
            ks, qs = pieces(pre(u['kb'][KSLOT[b], :, half])), pieces(u['qb'][jl])
        else:
            kb = cached(u, ('k', b), lambda: u['kb'][KSLOT[b]])
            qb = cached(u, ('q', lt), lambda: u['qb'][jl])
            ks = cached(u, ('k', b, half, w), lambda: pieces(kb[:, half]))
            qs = cached(u, ('q', lt, w), lambda: pieces(qb))
        acc = ks[0] * qs[0]
        if first is not None:
            acc = first(acc[0])[None]
        for k, q in zip(ks[1:], qs[1:]):
            acc = acc + k * q
        return acc[0] + acc[1] if w == 2 else acc[0]

    def qk(u, blks):
        if u['w'] is None:
            u['w'] = pltpu.bitcast(qt_scr[u['tq'], u['h']], BF16)
        kc = pltpu.bitcast(jnp.concatenate(blks, axis=0), BF16)[:, :DH]
        return jnp.dot(kc, u['w'], preferred_element_type=F32)

    def fast_step(jb, carry):
        flags = [flag_ref[k] > 0 for k in range(NFLAG)]

        def tie(x, dep, k=0):
            return lax.select(flags[k], x, dep if dep.dtype == x.dtype else pltpu.bitcast(dep, x.dtype))

        units = [unit(jb * 2 + i // NQ, i % NQ, i // NQ) for i in range(NUN)]
        units.append(unit(jnp.minimum(jb * 2 + 2, 2 * H - 1), 0, 0))
        sval = {m: cj_scr[m] for m in range(N_CJOB)}
        rows, popped, extra = {}, {}, {}
        for (t, r), n in CBLK_IDX.items():
            fin = jnp.exp2 if n >= len(CBLK) - CRAW else (lambda v: v)
            rows[(0, t, r)] = fin(cp_scr[n * 16:n * 16 + 8, :])
            rows[(0, t, r + 8)] = fin(cp_scr[n * 16 + 8:n * 16 + 16, :])

        chain = []

        def run_job(m, first=None):
            sval[m] = vjob(units[JOBS[m][0]], *JOBS[m][1:], first=first)
            if JOBS[m][0] == NUN:
                cj_scr[m - N_JOB] = sval[m]
            return sval[m]

        def operand(x, pos):
            due = []
            for fn, table, lag in ((bcast_k, KDL, KSTART), (bcast_q, QDL, QSTART)):
                for hh, it in table.get(pos, []):
                    src = popped[max(k for k in popped if k <= pos - lag)]
                    due.append(fn(units[(hh + 1) * NQ], *it, lambda v: tie(v, src)))
            if pos in XAT:
                chain.append(run_job(XAT[pos], lambda v: tie(v, chain[-1]) if chain else v))
                if pos + XLAG < W1:
                    extra.setdefault(pos + XLAG, []).append(chain[-1])
            if pos in JAT:
                due.append(run_job(JAT[pos]))
            due += extra.pop(pos, [])
            for k, dep in enumerate(due):
                x = tie(x, dep, k)
            return x

        def pv(i, t, pos):
            u = units[i]
            for r in range(0, VROWS[t], 8):
                rows[(i, t, r)] = jnp.exp2(
                    jnp.concatenate([sval[JIDX[(i, t, r, lt)]] for lt in range(NL)], axis=1))
            for r in range(120, -1, -8):
                u['l8'] = rows[(i, t, r)] if u['l8'] is None else u['l8'] + rows[(i, t, r)]
            pt = jnp.concatenate([rows.pop((i, t, r)) for r in range(0, 128, 8)], axis=0)
            vt = vt_scr[u['p'] * NQ + t // NL, u['h'], :, (t % NL) * 128:(t % NL + 1) * 128]
            o = jnp.dot(pltpu.bitcast(operand(vt, pos), BF16), pt, preferred_element_type=F32)
            u['acc'] = o if u['acc'] is None else u['acc'] + o
            if t == 0:
                for n in range(NL):
                    extra.setdefault(pos + FIRST + n, []).append(o[0:8, n * 128:(n + 1) * 128])
            if t == NT - 1:
                l = jnp.sum(u['l8'], axis=0, keepdims=True)
                r0 = pl.reciprocal(l, approx=True)
                r1 = r0 * (2.0 - l * r0)
                ot_scr[u['tq'], u['h']] = pltpu.bitcast((u['acc'] * r1).astype(BF16), U32)

        n = W0
        while n < W1:
            e = SEQ[n]
            if e[0] == 'P':
                pv(e[1], e[2], n)
                n += 1
                continue
            n1 = n
            while n1 < W1 and SEQ[n1][0] == 'K' and SEQ[n1][1] == e[1]:
                n1 += 1
            u = units[e[1]]
            blk = {}
            for t in sorted({SEQ[k][2] for k in range(n, n1)}):
                rs = [SEQ[k][3] for k in range(n, n1) if SEQ[k][2] == t]
                run = k_scr[u['ph'], (t * 128 + min(rs)) // 2:(t * 128 + max(rs)) // 2 + 8, :]
                for r in rs:
                    blk[(t, r)] = run[(r - min(rs)) // 2:(r - min(rs)) // 2 + 8]
            st = qk(u, [operand(blk[SEQ[k][2:]], k) for k in range(n, n1)])
            pm = jnp.exp2(st)
            for bi, k in enumerate(range(n, n1)):
                _, i, t, r = SEQ[k]
                if i == NUN:
                    c = CBLK_IDX[(t, r)]
                    cp_scr[c * 16:c * 16 + 16, :] = (st if c >= len(CBLK) - CRAW else pm)[bi * 16:bi * 16 + 16]
                else:
                    rows[(i, t, r)] = pm[bi * 16:bi * 16 + 8]
                    rows[(i, t, r + 8)] = pm[bi * 16 + 8:bi * 16 + 16]
                popped[k] = st[bi * 16:bi * 16 + 8, 0:128]
            n = n1
        for m in range(N_CJOB + N_JOB - HEAD, N_CJOB + N_JOB):
            run_job(m)
        return carry

    def slow_step(n, carry):
        u = unit(lax.shift_right_logical(n, 2), n & (NQ - 1), 0)
        w = pltpu.bitcast(qu_scr[u['tq'], u['h']], BF16)

        def scores(c):
            ku = k_scr[u['ph'], pl.ds(pl.multiple_of(c * (TQ // 2), TQ // 2), TQ // 2), :]
            blks = [ku[r // 2:r // 2 + 8] for r in range(0, TQ, 16)]
            blks = [pick(b * 16, c, lambda v=v: pltpu.bitcast(
                jnp.concatenate(split(v), axis=0).astype(BF16), U32), v) for b, v in enumerate(blks)]
            kc = pltpu.bitcast(jnp.concatenate(blks, axis=0), BF16)[:, :DH]
            s = jnp.dot(kc, w, preferred_element_type=F32)
            return s.astype(BF16).astype(F32) * DH ** -0.5

        m = lax.fori_loop(0, NQ, lambda c, m: jnp.maximum(m, jnp.max(scores(c), axis=0, keepdims=True)),
                          jnp.full((1, TQ), -jnp.inf, F32))

        def chunk(c, st):
            pt = jnp.exp((scores(c) - m).astype(BF16).astype(F32)).astype(BF16)
            vt = pltpu.bitcast(vt_scr[u['p'] * NQ + c, u['h']], BF16)
            return (st[0] + jnp.sum(pt.astype(F32), axis=0, keepdims=True),
                    st[1] + jnp.dot(vt, pt, preferred_element_type=F32))

        l, acc = lax.fori_loop(0, NQ, chunk, (jnp.zeros((1, TQ), F32), jnp.zeros((DH, TQ), F32)))
        ot_scr[u['tq'], u['h']] = pltpu.bitcast((acc / l).astype(BF16), U32)
        return carry

    u0 = unit(jnp.int32(0), 0, 0)
    st0 = qk(u0, [kblk(u0, e[2], e[3]) for e in CBLK])
    ne = (len(CBLK) - CRAW) * 16
    cp_scr[0:ne, :] = jnp.exp2(st0[0:ne])
    cp_scr[ne:, :] = st0[ne:]
    prev = pltpu.bitcast(ku_last[0:8, 0:128], F32)
    for m in range(N_CJOB):
        prev = vjob(u0, *JOBS[m][1:], pre=lambda v: jnp.where((flag_ref[0] > 0)[None], v, prev[None]))
        cj_scr[m] = prev

    @pl.when(safe)
    def _():
        lax.fori_loop(0, H, fast_step, 0)

    @pl.when(jnp.logical_not(safe))
    def _():
        lax.fori_loop(0, 2 * H * NQ, slow_step, 0)

    wo_copy(0).wait()
    wo_copy(1).wait()
    for t in range(2 * NQ):
        for s_ in range(TQ // TO):
            o_t = pltpu.bitcast(ot_scr[t, :, :, s_ * TO:(s_ + 1) * TO].reshape(H * 8, TO), BF16)
            out = lax.dot_general(o_t, wo_buf[t // NQ], (((0,), (0,)), ((), ())), preferred_element_type=F32)
            o_buf[t, s_ * TO:(s_ + 1) * TO, :] = out.astype(BF16)
            o_copy(t, s_).start()
    for t in range(2 * NQ):
        for s_ in range(TQ // TO):
            o_copy(t, s_).wait()


@jax.jit
def pallas_concat_heads__softmax_full_mha__softmax_full_mha__prompt_kernel(
    A_x: jax.Array,
    A_wqkv: jax.Array,
    A_wo: jax.Array,
    B_x: jax.Array,
    B_wqkv: jax.Array,
    B_wo: jax.Array,
):
    anyspec = pl.BlockSpec(memory_space=pl.ANY)
    return pl.pallas_call(
        _kernel,
        in_specs=[anyspec] * 6,
        out_specs=anyspec,
        out_shape=jax.ShapeDtypeStruct((1, S, 2 * D), BF16),
        scratch_shapes=[
            pltpu.VMEM((2 * NQ, TQ, D), BF16),
            pltpu.VMEM((6, D, D), BF16),
            pltpu.VMEM((2, D, D), BF16),
            pltpu.VMEM((2 * H, S // 2, 128), U32),
            pltpu.VMEM((2 * NQ, H, 8, TQ), U32),
            pltpu.VMEM((2 * NQ, H, 8, TQ), U32),
            pltpu.VMEM((2 * NQ, H, 8, TQ), U32),
            pltpu.VMEM((2 * NQ, H, NL, 2, 8, 128), F32),
            pltpu.VMEM((2 * NQ, H, 8, TQ), U32),
            pltpu.VMEM((2 * NQ * len(VREL), DH, 2, 8, 128), F32),
            pltpu.VMEM((NQ * len(VREL), DH, 2, 8, 128), F32),
            pltpu.VMEM((2 * NQ * NL, DH, 8, 128), F32),
            pltpu.VMEM((NQ * NL, DH, 8, 128), F32),
            pltpu.VMEM((len(CBLK) * 16, TQ), F32),
            pltpu.VMEM((N_CJOB, 8, 128), F32),
            pltpu.VMEM((H, TQ), F32),
            pltpu.VMEM((8, D), F32),
            pltpu.VMEM((2, 8, TQ), F32),
            pltpu.VMEM((NFLAG, 8, 128), jnp.int32),
            pltpu.SemaphoreType.DMA((2 * NQ,)),
            pltpu.SemaphoreType.DMA((6,)),
            pltpu.SemaphoreType.DMA((2,)),
            pltpu.SemaphoreType.DMA((2 * NQ * (TQ // TO),)),
        ],
        compiler_params=pltpu.CompilerParams(vmem_limit_bytes=96 * 1024 * 1024),
    )(A_x, A_wqkv, A_wo, B_x, B_wqkv, B_wo)
```
